```python
import jax
import jax.numpy as jnp

def _softmax(x, axis=-1):
    return jax.nn.softmax(x, axis=axis)
def _gelu(x):
    return jax.nn.gelu(x, approximate=True)
def _silu(x):
    return jax.nn.silu(x)
def _sigmoid(x):
    return jax.nn.sigmoid(x)
def _layernorm(x, axis=-1, eps=1e-5):
    m = jnp.mean(x, axis=axis, keepdims=True)
    v = jnp.var(x, axis=axis, keepdims=True)
    return (x - m) / jnp.sqrt(v + eps)
def _scatter_add(tgt, idx, src, axis=0):
    return tgt.at[idx].add(src)
def _segment_sum(src, seg, n):
    return jax.ops.segment_sum(src, seg, n)
class _Rng:
    def __init__(self, key):
        self._k = key
    def _next(self):
        self._k, sub = jax.random.split(self._k)
        return sub
    def normal(self, shape):
        return jax.random.normal(self._next(), shape, dtype=jnp.bfloat16)
    def randint(self, lo, hi, shape):
        return jax.random.randint(self._next(), shape, lo, hi, dtype=jnp.int32)
    def uniform(self, shape, lo=0.0, hi=1.0):
        return jax.random.uniform(self._next(), shape, jnp.bfloat16, lo, hi)
    def permutation(self, n):
        return jax.random.permutation(self._next(), n)


kernel_name = 'sequential_preLN__sliding_block_cached__mixer_s_mlp__decode'

def setup_inputs():
    _rng = _Rng(jax.random.key(int.from_bytes(__import__("os").urandom(4), "little")))
    _w = (lambda a: (lambda t: t.astype(jnp.bfloat16) if jnp.issubdtype(t.dtype, jnp.floating) else t)(jnp.asarray(a)))
    def _A_setup():
        B, Sq, D = 1, 1, 640
        Hq, Hkv, Sk, Dh = 32, 32, 32768, 192
        assert Hq % Hkv == 0, (Hq, Hkv)
        return {
            "x": _w((lambda *s: _rng.normal(s) * 0.05)(B, Sq, D)),
            "k_cache": _w((lambda *s: _rng.normal(s) * 0.05)(B, Hkv, Sk, Dh)),
            "v_cache": _w((lambda *s: _rng.normal(s) * 0.05)(B, Hkv, Sk, Dh)),
            "wq": _w((lambda *s: _rng.normal(s) * 0.05)(D, Hq * Dh) * (D ** -0.5)),
            "wo": _w((lambda *s: _rng.normal(s) * 0.05)(Hq * Dh, D) * ((Hq * Dh) ** -0.5)),
        }
    _A_in = _A_setup()

    def _B_setup():
        B, S, D, F = 1, 1, 640, 1536
        return {
            "x":  _w((lambda *s: _rng.normal(s) * 0.05)(B, S, D)),
            "w1": _w((lambda *s: _rng.normal(s) * 0.05)(D, D) * (D ** -0.5)),
            "w2": _w((lambda *s: _rng.normal(s) * 0.05)(D, D) * (D ** -0.5)),
            "w3": _w((lambda *s: _rng.normal(s) * 0.05)(D, F) * (D ** -0.5)),
            "w4": _w((lambda *s: _rng.normal(s) * 0.05)(F, D) * (F ** -0.5)),
        }
    _B_in = _B_setup()

    return {
        "A_x": _A_in["x"],
        "A_k_cache": _A_in["k_cache"],
        "A_v_cache": _A_in["v_cache"],
        "A_wq": _A_in["wq"],
        "A_wo": _A_in["wo"],
        "B_x": _B_in["x"],
        "B_w1": _B_in["w1"],
        "B_w2": _B_in["w2"],
        "B_w3": _B_in["w3"],
        "B_w4": _B_in["w4"],
    }

def reference(A_x, A_k_cache, A_v_cache, A_wq, A_wo, B_x, B_w1, B_w2, B_w3, B_w4):
    def _A_ref(x, k_cache, v_cache, wq, wo):
        B, Sq, D = x.shape
        Hq, Dh = 32, 192
        Hkv, Sk = k_cache.shape[1], k_cache.shape[2]
        W = min(4096, max(256, Sk // 4))
        rep = Hq // Hkv
        q = (lambda x, *d: x.transpose(*d))((x @ wq).reshape(B, Sq, Hq, Dh), 0, 2, 1, 3)
        k = jnp.repeat(k_cache[:, :, Sk - W:, :], rep, axis=1)
        v = jnp.repeat(v_cache[:, :, Sk - W:, :], rep, axis=1)
        scores = jnp.einsum("bhqd,bhkd->bhqk", q, k) * (Dh ** -0.5)
        p = _softmax(scores, axis=-1)
        o = jnp.einsum("bhqk,bhkd->bhqd", p, v)
        return (lambda x, *d: x.transpose(*d))(o, 0, 2, 1, 3).reshape(B, Sq, Hq * Dh) @ wo

    def _B_ref(x, w1, w2, w3, w4):
        B, S, D = x.shape
        h = _gelu(_layernorm(x, axis=-1) @ w1)
        c = D // 4
        g0 = jnp.pad(h[:, :, 0*c:1*c], ((0, 0), (1, 0), (0, 0)))[:, :S, :]
        g1 = jnp.pad(h[:, :, 1*c:2*c], ((0, 0), (0, 1), (0, 0)))[:, 1:, :]
        g2 = jnp.pad(h[:, :, 2*c:3*c], ((0, 0), (2, 0), (0, 0)))[:, :S, :]
        g3 = jnp.pad(h[:, :, 3*c:   ], ((0, 0), (0, 2), (0, 0)))[:, 2:, :]
        hs = jnp.concatenate([g0, g1, g2, g3], axis=-1) @ w2
        x1 = x + hs
        h2 = _gelu(_layernorm(x1, axis=-1) @ w3) @ w4
        return x1 + h2

    x = A_x
    h = x + _A_ref(_layernorm(x, axis=-1), A_k_cache, A_v_cache, A_wq, A_wo)
    h2 = h + _B_ref(_layernorm(h, axis=-1), B_w1, B_w2, B_w3, B_w4)
    return h2
```

```python
import jax
import jax.numpy as jnp
from jax import lax
import jax.experimental.pallas as pl
import jax.experimental.pallas.tpu as pltpu

_EPS = 1e-5


def _layernorm(x):
    m = jnp.mean(x, axis=-1, keepdims=True)
    d = x - m
    v = jnp.mean(d * d, axis=-1, keepdims=True)
    return d / jnp.sqrt(v + _EPS)


@jax.jit
def pallas_sequential_preLN__sliding_block_cached__mixer_s_mlp__decode_kernel(
    A_x: jax.Array,
    A_k_cache: jax.Array,
    A_v_cache: jax.Array,
    A_wq: jax.Array,
    A_wo: jax.Array,
    B_x: jax.Array,
    B_w1: jax.Array,
    B_w2: jax.Array,
    B_w3: jax.Array,
    B_w4: jax.Array,
):
    B, Sq, D = A_x.shape
    Hq, Dh = 32, 192
    Hkv, Sk = A_k_cache.shape[1], A_k_cache.shape[2]
    F = B_w3.shape[1]
    assert B == 1 and Sq == 1 and Hkv == Hq
    W = min(4096, max(256, Sk // 4))
    R = Hq * Dh
    PR = 2 * Dh
    NP = Hq // 2
    NB = 4
    M = 8
    QC = 4
    QW = R // QC
    OC = 4
    OW = R // OC
    C3 = 3
    W3 = F // C3
    w4_rows = [512, 512, 384, 128]
    w4_off = [sum(w4_rows[:i]) for i in range(len(w4_rows))]
    scale = Dh ** -0.5
    bf16, f32 = jnp.bfloat16, jnp.float32

    kT = A_k_cache.transpose(0, 1, 3, 2).reshape(R, Sk)
    vT = A_v_cache.transpose(0, 1, 3, 2).reshape(R, Sk)
    x2 = A_x.reshape(Sq, D)

    def kernel(x_hbm, k_hbm, v_hbm, wq_hbm, wo_hbm, w3_hbm, w4_hbm, out_ref,
               x_v, wq_v, wo_v, w3_v, w4_v, kbuf, vbuf, q_scr, o_scr,
               sem_x, sem_wq, sem_wo, sem_w3, sem_w4, sem_k, sem_v):

        def x_cp():
            return pltpu.make_async_copy(x_hbm, x_v, sem_x.at[0])

        def wq_cp(c):
            return pltpu.make_async_copy(
                wq_hbm.at[:, pl.ds(c * QW, QW)], wq_v.at[c], sem_wq.at[c])

        def k_cp(p, slot):
            return pltpu.make_async_copy(
                k_hbm.at[pl.ds(p * PR, PR), pl.ds(Sk - W, W)],
                kbuf.at[slot], sem_k.at[slot])

        def v_cp(p, slot):
            return pltpu.make_async_copy(
                v_hbm.at[pl.ds(p * PR, PR), pl.ds(Sk - W, W)],
                vbuf.at[slot], sem_v.at[slot])

        def wo_cp(c):
            return pltpu.make_async_copy(
                wo_hbm.at[pl.ds(c * OW, OW), :], wo_v.at[c], sem_wo.at[c])

        def w3_cp(c):
            return pltpu.make_async_copy(
                w3_hbm.at[:, pl.ds(c * W3, W3)], w3_v.at[c], sem_w3.at[c])

        def w4_cp(c):
            return pltpu.make_async_copy(
                w4_hbm.at[pl.ds(w4_off[c], w4_rows[c]), :],
                w4_v.at[pl.ds(w4_off[c], w4_rows[c]), :], sem_w4.at[c])

        tail = ([lambda c=c: wo_cp(c) for c in range(OC)]
                + [lambda c=c: w3_cp(c) for c in range(C3)]
                + [lambda c=c: w4_cp(c) for c in range(len(w4_rows))])
        TA = 2 * NB

        x_cp().start()
        for c in range(QC):
            wq_cp(c).start()
        for p in range(NB):
            k_cp(p, p).start()
            v_cp(p, p).start()

        x_cp().wait()
        xf = x_v[...].astype(f32)
        xn = jnp.broadcast_to(_layernorm(xf), (M, D)).astype(bf16)

        row = lax.broadcasted_iota(jnp.int32, (M, PR), 0)
        lane = lax.broadcasted_iota(jnp.int32, (M, PR), 1)
        diag = jnp.logical_or(jnp.logical_and(row == 0, lane < Dh),
                              jnp.logical_and(row == 1, lane >= Dh))

        for c in range(QC):
            wq_cp(c).wait()
            q = jnp.dot(xn, wq_v[c], preferred_element_type=f32)
            for j in range(QW // PR):
                qj = q[:, j * PR:(j + 1) * PR]
                q_scr[c * (QW // PR) + j] = jnp.where(diag, qj, 0.0).astype(bf16)

        def pair(p, carry):
            slot = p % NB
            k_cp(p, slot).wait()
            s = jnp.dot(q_scr[p], kbuf[slot], preferred_element_type=f32)

            @pl.when(p + NB < NP)
            def _():
                k_cp(p + NB, slot).start()

            for t in range(NB):
                @pl.when(p + NB == NP + t)
                def _():
                    tail[2 * t]().start()

            s = s * scale
            m = jnp.max(s, axis=-1, keepdims=True)
            e = jnp.exp(s - m)
            l = jnp.sum(e, axis=-1, keepdims=True)

            v_cp(p, slot).wait()
            o = lax.dot_general(e.astype(bf16), vbuf[slot],
                                (((1,), (1,)), ((), ())),
                                preferred_element_type=f32)

            @pl.when(p + NB < NP)
            def _():
                v_cp(p + NB, slot).start()

            for t in range(NB):
                @pl.when(p + NB == NP + t)
                def _():
                    tail[2 * t + 1]().start()

            o_scr[p] = jnp.where(diag, o / l, 0.0).astype(bf16)
            return carry

        lax.fori_loop(0, NP, pair, 0)

        nxt = [TA]

        def issue_next():
            if nxt[0] < len(tail):
                tail[nxt[0]]().start()
                nxt[0] += 1

        acc = jnp.zeros((M, D), f32)
        ppc = OW // PR
        for c in range(OC):
            wo_cp(c).wait()
            oc = jnp.concatenate([o_scr[c * ppc + j] for j in range(ppc)], axis=-1)
            acc = acc + jnp.dot(oc, wo_v[c], preferred_element_type=f32)
            issue_next()
        attn = jnp.sum(acc, axis=0, keepdims=True)
        h = xf + attn
        x1 = _layernorm(h)
        x1n = jnp.broadcast_to(_layernorm(x1), (M, D)).astype(bf16)
        g = []
        for c in range(C3):
            w3_cp(c).wait()
            u = jnp.dot(x1n, w3_v[c], preferred_element_type=f32)
            g.append(jax.nn.gelu(u, approximate=True).astype(bf16))
            issue_next()
        g = jnp.concatenate(g, axis=-1)
        y = jnp.zeros((M, D), f32)
        for c in range(len(w4_rows)):
            w4_cp(c).wait()
            r0, rn = w4_off[c], w4_rows[c]
            y = y + jnp.dot(g[:, r0:r0 + rn], w4_v[r0:r0 + rn, :],
                            preferred_element_type=f32)
            issue_next()
        out_ref[...] = (h + (x1 + y[0:1, :])).astype(out_ref.dtype)

    any_spec = pl.BlockSpec(memory_space=pl.ANY)
    out = pl.pallas_call(
        kernel,
        out_shape=jax.ShapeDtypeStruct((Sq, D), A_x.dtype),
        in_specs=[any_spec] * 7,
        out_specs=pl.BlockSpec(memory_space=pltpu.VMEM),
        scratch_shapes=[
            pltpu.VMEM((Sq, D), bf16),
            pltpu.VMEM((QC, D, QW), bf16),
            pltpu.VMEM((OC, OW, D), bf16),
            pltpu.VMEM((C3, D, W3), bf16),
            pltpu.VMEM((F, D), bf16),
            pltpu.VMEM((NB, PR, W), bf16),
            pltpu.VMEM((NB, PR, W), bf16),
            pltpu.VMEM((NP, M, PR), bf16),
            pltpu.VMEM((NP, M, PR), bf16),
            pltpu.SemaphoreType.DMA((1,)),
            pltpu.SemaphoreType.DMA((QC,)),
            pltpu.SemaphoreType.DMA((OC,)),
            pltpu.SemaphoreType.DMA((C3,)),
            pltpu.SemaphoreType.DMA((len(w4_rows),)),
            pltpu.SemaphoreType.DMA((NB,)),
            pltpu.SemaphoreType.DMA((NB,)),
        ],
        compiler_params=pltpu.CompilerParams(
            vmem_limit_bytes=100 * 1024 * 1024,
        ),
    )(x2, kT, vT, A_wq, A_wo, B_w3, B_w4)
    return out.reshape(B, Sq, D)
```

```python
import jax
import jax.numpy as jnp
from jax import lax
import jax.experimental.pallas as pl
import jax.experimental.pallas.tpu as pltpu

_EPS = 1e-5


def _layernorm(x):
    m = jnp.mean(x, axis=-1, keepdims=True)
    d = x - m
    v = jnp.mean(d * d, axis=-1, keepdims=True)
    return d / jnp.sqrt(v + _EPS)


@jax.jit
def pallas_sequential_preLN__sliding_block_cached__mixer_s_mlp__decode_kernel(
    A_x: jax.Array,
    A_k_cache: jax.Array,
    A_v_cache: jax.Array,
    A_wq: jax.Array,
    A_wo: jax.Array,
    B_x: jax.Array,
    B_w1: jax.Array,
    B_w2: jax.Array,
    B_w3: jax.Array,
    B_w4: jax.Array,
):
    B, Sq, D = A_x.shape
    Hq, Dh = 32, 192
    Hkv, Sk = A_k_cache.shape[1], A_k_cache.shape[2]
    F = B_w3.shape[1]
    assert B == 1 and Sq == 1 and Hkv == Hq and Hq % 2 == 0
    W = min(4096, max(256, Sk // 4))
    R = Hq * Dh
    PR = 2 * Dh
    NP = Hq // 2
    S = 4
    M = 8
    QC = 4
    QW = R // QC
    OC = 4
    OW = R // OC
    C3 = 3
    W3 = F // C3
    w4_rows = [512, 512, 384, 128]
    w4_off = [sum(w4_rows[:i]) for i in range(len(w4_rows))]
    assert sum(w4_rows) == F and S % 2 == 0
    KV0 = 1 + QC
    T0 = KV0 + 2 * NP
    scale = Dh ** -0.5
    bf16, f32 = jnp.bfloat16, jnp.float32

    kT = A_k_cache.transpose(0, 1, 3, 2).reshape(R, Sk)
    vT = A_v_cache.transpose(0, 1, 3, 2).reshape(R, Sk)
    x2 = A_x.reshape(Sq, D)

    def kernel(x_hbm, k_hbm, v_hbm, wq_hbm, wo_hbm, w3_hbm, w4_hbm, out_ref,
               x_v, wq_v, wo_v, w3_v, w4_v, ring, q_scr, o_scr, sems):

        def kv_copy(src, p, slot):
            return pltpu.make_async_copy(
                src.at[pl.ds(p * PR, PR), pl.ds(Sk - W, W)],
                ring.at[slot], sems.at[slot])

        tail = ([(wo_hbm.at[pl.ds(c * OW, OW), :], wo_v.at[c]) for c in range(OC)]
                + [(w3_hbm.at[:, pl.ds(c * W3, W3)], w3_v.at[c]) for c in range(C3)]
                + [(w4_hbm.at[pl.ds(r0, rn), :], w4_v.at[pl.ds(r0, rn), :])
                   for r0, rn in zip(w4_off, w4_rows)])
        NT = T0 + len(tail)

        def copy(i):
            sem = sems.at[i % S]
            if i == 0:
                return pltpu.make_async_copy(x_hbm, x_v, sem)
            if i < KV0:
                c = i - 1
                return pltpu.make_async_copy(
                    wq_hbm.at[:, pl.ds(c * QW, QW)], wq_v.at[c], sem)
            if i < T0:
                j = i - KV0
                return kv_copy(k_hbm if j % 2 == 0 else v_hbm, j // 2, i % S)
            return pltpu.make_async_copy(*tail[i - T0], sem)

        def advance(i):
            copy(i).wait()
            if i + S < NT:
                copy(i + S).start()

        for i in range(S):
            copy(i).start()

        advance(0)
        xf = x_v[...].astype(f32)
        xn = jnp.broadcast_to(_layernorm(xf), (M, D)).astype(bf16)

        row = lax.broadcasted_iota(jnp.int32, (M, PR), 0)
        lane = lax.broadcasted_iota(jnp.int32, (M, PR), 1)
        diag = jnp.logical_or(jnp.logical_and(row == 0, lane < Dh),
                              jnp.logical_and(row == 1, lane >= Dh))

        for c in range(QC):
            advance(1 + c)
            q = jnp.dot(xn, wq_v[c], preferred_element_type=f32)
            for j in range(QW // PR):
                q_scr[c * (QW // PR) + j] = jnp.where(
                    diag, q[:, j * PR:(j + 1) * PR], 0.0).astype(bf16)

        def refill(p, kv, slot):
            src = k_hbm if kv == 0 else v_hbm
            pn = p + S // 2

            @pl.when(pn < NP)
            def _():
                kv_copy(src, pn, slot).start()

            for t in range(kv, S, 2):
                @pl.when(p == (2 * NP + t - kv - S) // 2)
                def _():
                    copy(T0 + t).start()

        def pair(p, carry):
            ks = (KV0 + 2 * p) % S
            vs = (KV0 + 2 * p + 1) % S
            kv_copy(k_hbm, p, ks).wait()
            s = jnp.dot(q_scr[p], ring[ks], preferred_element_type=f32)
            refill(p, 0, ks)
            s = s * scale
            m = jnp.max(s, axis=-1, keepdims=True)
            e = jnp.exp(s - m)
            l = jnp.sum(e, axis=-1, keepdims=True)
            kv_copy(v_hbm, p, vs).wait()
            o = lax.dot_general(e.astype(bf16), ring[vs],
                                (((1,), (1,)), ((), ())),
                                preferred_element_type=f32)
            refill(p, 1, vs)
            o_scr[p] = jnp.where(diag, o / l, 0.0).astype(bf16)
            return carry

        lax.fori_loop(0, NP, pair, 0)

        i = T0
        acc = jnp.zeros((M, D), f32)
        ppc = OW // PR
        for c in range(OC):
            advance(i)
            i += 1
            oc = jnp.concatenate([o_scr[c * ppc + j] for j in range(ppc)], axis=-1)
            acc = acc + jnp.dot(oc, wo_v[c], preferred_element_type=f32)
        h = xf + jnp.sum(acc, axis=0, keepdims=True)

        x1 = _layernorm(h)
        x1n = jnp.broadcast_to(_layernorm(x1), (M, D)).astype(bf16)
        g = []
        for c in range(C3):
            advance(i)
            i += 1
            u = jnp.dot(x1n, w3_v[c], preferred_element_type=f32)
            g.append(jax.nn.gelu(u, approximate=True).astype(bf16))
        g = jnp.concatenate(g, axis=-1)
        y = jnp.zeros((M, D), f32)
        for r0, rn in zip(w4_off, w4_rows):
            advance(i)
            i += 1
            y = y + jnp.dot(g[:, r0:r0 + rn], w4_v[r0:r0 + rn, :],
                            preferred_element_type=f32)
        out_ref[...] = (h + (x1 + y[0:1, :])).astype(out_ref.dtype)

    out = pl.pallas_call(
        kernel,
        out_shape=jax.ShapeDtypeStruct((Sq, D), A_x.dtype),
        in_specs=[pl.BlockSpec(memory_space=pl.ANY)] * 7,
        out_specs=pl.BlockSpec(memory_space=pltpu.VMEM),
        scratch_shapes=[
            pltpu.VMEM((Sq, D), bf16),
            pltpu.VMEM((QC, D, QW), bf16),
            pltpu.VMEM((OC, OW, D), bf16),
            pltpu.VMEM((C3, D, W3), bf16),
            pltpu.VMEM((F, D), bf16),
            pltpu.VMEM((S, PR, W), bf16),
            pltpu.VMEM((NP, M, PR), bf16),
            pltpu.VMEM((NP, M, PR), bf16),
            pltpu.SemaphoreType.DMA((S,)),
        ],
        compiler_params=pltpu.CompilerParams(vmem_limit_bytes=64 * 1024 * 1024),
    )(x2, kT, vT, A_wq, A_wo, B_w3, B_w4)
    return out.reshape(B, Sq, D)
```

```python
import jax
import jax.numpy as jnp
from jax import lax
import jax.experimental.pallas as pl
import jax.experimental.pallas.tpu as pltpu

_EPS = 1e-5


def _layernorm(x):
    m = jnp.mean(x, axis=-1, keepdims=True)
    d = x - m
    v = jnp.mean(d * d, axis=-1, keepdims=True)
    return d / jnp.sqrt(v + _EPS)


@jax.jit
def pallas_sequential_preLN__sliding_block_cached__mixer_s_mlp__decode_kernel(
    A_x: jax.Array,
    A_k_cache: jax.Array,
    A_v_cache: jax.Array,
    A_wq: jax.Array,
    A_wo: jax.Array,
    B_x: jax.Array,
    B_w1: jax.Array,
    B_w2: jax.Array,
    B_w3: jax.Array,
    B_w4: jax.Array,
):
    B, Sq, D = A_x.shape
    Hq, Dh = 32, 192
    Hkv, Sk = A_k_cache.shape[1], A_k_cache.shape[2]
    F = B_w3.shape[1]
    assert B == 1 and Sq == 1 and Hkv == Hq and Hq % 2 == 0
    W = min(4096, max(256, Sk // 4))
    R = Hq * Dh
    PR = 2 * Dh
    NP = Hq // 2
    S = 4
    M = 8
    QC = 4
    QW = R // QC
    OC = 4
    OW = R // OC
    C3 = 3
    W3 = F // C3
    w4_mxu = [512, 512, 256, 128]
    w4_vpu = [64, 64]
    w4_rows = w4_mxu + w4_vpu
    w4_off = [sum(w4_rows[:i]) for i in range(len(w4_rows))]
    V0 = sum(w4_mxu)
    assert sum(w4_rows) == F and F - V0 == 128 and D % 128 == 0 and S % 2 == 0
    KV0 = 1 + QC
    T0 = KV0 + 2 * NP
    scale = Dh ** -0.5
    bf16, f32 = jnp.bfloat16, jnp.float32

    kT = A_k_cache.transpose(0, 1, 3, 2).reshape(R, Sk)
    vT = A_v_cache.transpose(0, 1, 3, 2).reshape(R, Sk)
    x2 = A_x.reshape(Sq, D)

    def kernel(x_hbm, k_hbm, v_hbm, wq_hbm, wo_hbm, w3_hbm, w4_hbm, out_ref,
               x_v, wq_v, wo_v, w3_v, ring, q_scr, o_scr, sems, *w4_v):

        def kv_copy(src, p, slot):
            return pltpu.make_async_copy(
                src.at[pl.ds(p * PR, PR), pl.ds(Sk - W, W)],
                ring.at[slot], sems.at[slot])

        tail = ([(wo_hbm.at[pl.ds(c * OW, OW), :], wo_v.at[c]) for c in range(OC)]
                + [(w3_hbm.at[:, pl.ds(c * W3, W3)], w3_v.at[c]) for c in range(C3)]
                + [(w4_hbm.at[pl.ds(r0, rn), :], buf)
                   for r0, rn, buf in zip(w4_off, w4_rows, w4_v)])
        NT = T0 + len(tail)

        def copy(i):
            sem = sems.at[i % S]
            if i == 0:
                return pltpu.make_async_copy(x_hbm, x_v, sem)
            if i < KV0:
                c = i - 1
                return pltpu.make_async_copy(
                    wq_hbm.at[:, pl.ds(c * QW, QW)], wq_v.at[c], sem)
            if i < T0:
                j = i - KV0
                return kv_copy(k_hbm if j % 2 == 0 else v_hbm, j // 2, i % S)
            return pltpu.make_async_copy(*tail[i - T0], sem)

        def advance(i):
            copy(i).wait()
            if i + S < NT:
                copy(i + S).start()

        for i in range(S):
            copy(i).start()

        advance(0)
        xf = x_v[...].astype(f32)
        xn = jnp.broadcast_to(_layernorm(xf), (M, D)).astype(bf16)

        row = lax.broadcasted_iota(jnp.int32, (M, PR), 0)
        lane = lax.broadcasted_iota(jnp.int32, (M, PR), 1)
        diag = jnp.logical_or(jnp.logical_and(row == 0, lane < Dh),
                              jnp.logical_and(row == 1, lane >= Dh))

        for c in range(QC):
            advance(1 + c)
            q = jnp.dot(xn, wq_v[c], preferred_element_type=f32)
            for j in range(QW // PR):
                q_scr[c * (QW // PR) + j] = jnp.where(
                    diag, q[:, j * PR:(j + 1) * PR], 0.0).astype(bf16)

        def refill(p, kv, slot):
            src = k_hbm if kv == 0 else v_hbm
            pn = p + S // 2

            @pl.when(pn < NP)
            def _():
                kv_copy(src, pn, slot).start()

            for t in range(kv, S, 2):
                @pl.when(p == (2 * NP + t - kv - S) // 2)
                def _():
                    copy(T0 + t).start()

        def pair(p, carry):
            ks = (KV0 + 2 * p) % S
            vs = (KV0 + 2 * p + 1) % S
            kv_copy(k_hbm, p, ks).wait()
            s = jnp.dot(q_scr[p], ring[ks], preferred_element_type=f32)
            refill(p, 0, ks)
            s = s * scale
            m = jnp.max(s, axis=-1, keepdims=True)
            e = jnp.exp(s - m)
            l = jnp.sum(e, axis=-1, keepdims=True)
            kv_copy(v_hbm, p, vs).wait()
            o = lax.dot_general(e.astype(bf16), ring[vs],
                                (((1,), (1,)), ((), ())),
                                preferred_element_type=f32)
            refill(p, 1, vs)
            o_scr[p] = jnp.where(diag, o / l, 0.0).astype(bf16)
            return carry

        lax.fori_loop(0, NP, pair, 0)

        i = T0
        acc = jnp.zeros((M, D), f32)
        ppc = OW // PR
        for c in range(OC):
            advance(i)
            i += 1
            oc = jnp.concatenate([o_scr[c * ppc + j] for j in range(ppc)], axis=-1)
            acc = acc + jnp.dot(oc, wo_v[c], preferred_element_type=f32)
        h = xf + jnp.sum(acc, axis=0, keepdims=True)

        x1 = _layernorm(h)
        x1n = jnp.broadcast_to(_layernorm(x1), (M, D)).astype(bf16)
        g = []
        for c in range(C3):
            advance(i)
            i += 1
            u = jnp.dot(x1n, w3_v[c], preferred_element_type=f32)
            g.append(jax.nn.gelu(u, approximate=True))
        g = jnp.concatenate(g, axis=-1)
        gb = g.astype(bf16)
        gcol = jnp.transpose(jnp.broadcast_to(g[0:1, V0:], (128, 128)))

        y = jnp.zeros((M, D), f32)
        yv = []
        for r0, rn, buf in zip(w4_off, w4_rows, w4_v):
            advance(i)
            i += 1
            w = buf[...]
            if r0 < V0:
                y = y + jnp.dot(gb[:, r0:r0 + rn], w, preferred_element_type=f32)
                if r0 + rn == V0:
                    base = h + (x1 + y[0:1, :])
            else:
                gc = gcol[r0 - V0:r0 - V0 + rn, :]
                prod = w.astype(f32) * jnp.concatenate([gc] * (D // 128), axis=1)
                yv.append(prod.reshape(rn // 8, 8, D).sum(axis=0))
        rest = jnp.sum(sum(yv[1:], yv[0]), axis=0, keepdims=True)
        out_ref[...] = (base + rest).astype(out_ref.dtype)

    out = pl.pallas_call(
        kernel,
        out_shape=jax.ShapeDtypeStruct((Sq, D), A_x.dtype),
        in_specs=[pl.BlockSpec(memory_space=pl.ANY)] * 7,
        out_specs=pl.BlockSpec(memory_space=pltpu.VMEM),
        scratch_shapes=[
            pltpu.VMEM((Sq, D), bf16),
            pltpu.VMEM((QC, D, QW), bf16),
            pltpu.VMEM((OC, OW, D), bf16),
            pltpu.VMEM((C3, D, W3), bf16),
            pltpu.VMEM((S, PR, W), bf16),
            pltpu.VMEM((NP, M, PR), bf16),
            pltpu.VMEM((NP, M, PR), bf16),
            pltpu.SemaphoreType.DMA((S,)),
        ] + [pltpu.VMEM((rn, D), bf16) for rn in w4_rows],
        compiler_params=pltpu.CompilerParams(vmem_limit_bytes=64 * 1024 * 1024),
    )(x2, kT, vT, A_wq, A_wo, B_w3, B_w4)
    return out.reshape(B, Sq, D)
```
